```python
import os as _os
_os.environ.setdefault("JAX_PLATFORMS", "cpu")
import jax
import jax.numpy as jnp

def _softmax(x, axis=-1):
    return jax.nn.softmax(x, axis=axis)
def _gelu(x):
    return jax.nn.gelu(x, approximate=True)
def _silu(x):
    return jax.nn.silu(x)
def _sigmoid(x):
    return jax.nn.sigmoid(x)
def _layernorm(x, axis=-1, eps=1e-5):
    m = jnp.mean(x, axis=axis, keepdims=True)
    v = jnp.var(x, axis=axis, keepdims=True)
    return (x - m) / jnp.sqrt(v + eps)
def _scatter_add(tgt, idx, src, axis=0):
    return tgt.at[idx].add(src)
def _segment_sum(src, seg, n):
    return jax.ops.segment_sum(src, seg, n)
class _Rng:
    def __init__(self, key):
        self._k = key
    def _next(self):
        self._k, sub = jax.random.split(self._k)
        return sub
    def normal(self, shape):
        return jax.random.normal(self._next(), shape, dtype=jnp.bfloat16)
    def randint(self, lo, hi, shape):
        return jax.random.randint(self._next(), shape, lo, hi, dtype=jnp.int32)
    def uniform(self, shape, lo=0.0, hi=1.0):
        return jax.random.uniform(self._next(), shape, jnp.bfloat16, lo, hi)
    def permutation(self, n):
        return jax.random.permutation(self._next(), n)


kernel_name = 'concat_heads__gqa_block_cached__gqa_block_cached__near_ridge'

def setup_inputs():
    _rng = _Rng(jax.random.key(int.from_bytes(__import__("os").urandom(4), "little")))
    _w = (lambda a: (lambda t: t.astype(jnp.bfloat16) if jnp.issubdtype(t.dtype, jnp.floating) else t)(jnp.asarray(a)))
    def _A_setup():
        B, Sq, D = 8, 240, 640
        Hq, Hkv, Sk, Dh = 32, 32, 1024, 192
        assert Hq % Hkv == 0, (Hq, Hkv)
        return {
            "x": _w((lambda *s: _rng.normal(s) * 0.8)(B, Sq, D)),
            "k_cache": _w((lambda *s: _rng.normal(s) * 0.8)(B, Hkv, Sk, Dh)),
            "v_cache": _w((lambda *s: _rng.normal(s) * 0.05)(B, Hkv, Sk, Dh)),
            "wq": _w((lambda *s: _rng.normal(s) * 0.8)(D, Hq * Dh) * (D ** -0.5)),
            "wo": _w((lambda *s: _rng.normal(s) * 0.05)(Hq * Dh, D) * ((Hq * Dh) ** -0.5)),
        }
    _A_in = _A_setup()

    def _B_setup():
        B, Sq, D = 8, 240, 640
        Hq, Hkv, Sk, Dh = 32, 32, 1024, 192
        assert Hq % Hkv == 0, (Hq, Hkv)
        return {
            "x": _w((lambda *s: _rng.normal(s) * 0.8)(B, Sq, D)),
            "k_cache": _w((lambda *s: _rng.normal(s) * 0.8)(B, Hkv, Sk, Dh)),
            "v_cache": _w((lambda *s: _rng.normal(s) * 0.05)(B, Hkv, Sk, Dh)),
            "wq": _w((lambda *s: _rng.normal(s) * 0.8)(D, Hq * Dh) * (D ** -0.5)),
            "wo": _w((lambda *s: _rng.normal(s) * 0.05)(Hq * Dh, D) * ((Hq * Dh) ** -0.5)),
        }
    _B_in = _B_setup()

    return {
        "A_x": _A_in["x"],
        "A_k_cache": _A_in["k_cache"],
        "A_v_cache": _A_in["v_cache"],
        "A_wq": _A_in["wq"],
        "A_wo": _A_in["wo"],
        "B_x": _B_in["x"],
        "B_k_cache": _B_in["k_cache"],
        "B_v_cache": _B_in["v_cache"],
        "B_wq": _B_in["wq"],
        "B_wo": _B_in["wo"],
    }

def reference(A_x, A_k_cache, A_v_cache, A_wq, A_wo, B_x, B_k_cache, B_v_cache, B_wq, B_wo):
    def _A_ref(x, k_cache, v_cache, wq, wo):
        B, Sq, D = x.shape
        Hq, Dh = 32, 192
        Hkv = k_cache.shape[1]
        rep = Hq // Hkv
        q = (lambda x, *d: x.transpose(*d))((x @ wq).reshape(B, Sq, Hq, Dh), 0, 2, 1, 3)
        k = jnp.repeat(k_cache, rep, axis=1)
        v = jnp.repeat(v_cache, rep, axis=1)
        scores = jnp.einsum("bhqd,bhkd->bhqk", q, k) * (Dh ** -0.5)
        p = _softmax(scores, axis=-1)
        o = jnp.einsum("bhqk,bhkd->bhqd", p, v)
        return (lambda x, *d: x.transpose(*d))(o, 0, 2, 1, 3).reshape(B, Sq, Hq * Dh) @ wo

    def _B_ref(x, k_cache, v_cache, wq, wo):
        B, Sq, D = x.shape
        Hq, Dh = 32, 192
        Hkv = k_cache.shape[1]
        rep = Hq // Hkv
        q = (lambda x, *d: x.transpose(*d))((x @ wq).reshape(B, Sq, Hq, Dh), 0, 2, 1, 3)
        k = jnp.repeat(k_cache, rep, axis=1)
        v = jnp.repeat(v_cache, rep, axis=1)
        scores = jnp.einsum("bhqd,bhkd->bhqk", q, k) * (Dh ** -0.5)
        p = _softmax(scores, axis=-1)
        o = jnp.einsum("bhqk,bhkd->bhqd", p, v)
        return (lambda x, *d: x.transpose(*d))(o, 0, 2, 1, 3).reshape(B, Sq, Hq * Dh) @ wo

    a = _A_ref(A_x, A_k_cache, A_v_cache, A_wq, A_wo)
    b = _B_ref(B_x, B_k_cache, B_v_cache, B_wq, B_wo)
    return jnp.concatenate([a, b], axis=-1)
```

```python
import functools

import jax
import jax.numpy as jnp
from jax import lax
import jax.experimental.pallas as pl
import jax.experimental.pallas.tpu as pltpu

_B, _SQ, _D, _H, _SK, _DH = 8, 240, 640, 32, 1024, 192
_NP = _H // 2
_PW = 2 * _DH
_NTASK = _NP * _B
_T = 2
_NS = 2

_LOG2E = 1.4426950408889634
_QSCALE = _DH ** -0.5 * _LOG2E
_NT = (((1,), (1,)), ((), ()))
_F32 = jnp.float32
_BF16 = jnp.bfloat16


def _qproj(x, wq):
    q = jnp.dot(x, wq, preferred_element_type=_F32) * _QSCALE
    lane = lax.broadcasted_iota(jnp.int32, (_SQ, 128), 1)
    t0, t1, t2 = q[:, 0:128], q[:, 128:256], q[:, 256:384]
    q0 = jnp.concatenate([t0, jnp.where(lane < 64, t1, 0.0)], axis=1)
    q1 = jnp.concatenate([jnp.where(lane >= 64, t1, 0.0), t2], axis=1)
    return q0.astype(_BF16), q1.astype(_BF16)


def _scores(q, k_ref, h):
    return jnp.dot(q, k_ref[128 * h:128 * h + 256], preferred_element_type=_F32)


def _softmax(s):
    m = jnp.max(s, axis=-1, keepdims=True)
    p = jnp.exp2(s - m).astype(_BF16)
    l = jnp.sum(p.astype(_F32), axis=-1, keepdims=True)
    r = pl.reciprocal(l, approx=True)
    r = r * (2.0 - l * r)
    return p, r


def _pv(p, v_ref, h):
    if h == 0:
        vn, vt = v_ref[0:128], v_ref[128:192]
    else:
        vt, vn = v_ref[192:256], v_ref[256:384]
    on = lax.dot_general(p, vn, _NT, preferred_element_type=_F32)
    ot = lax.dot_general(vt, p, _NT, preferred_element_type=_F32)
    return on, ot


def _oproj(o0, o1, r0, r1, wo):
    on0, ot0 = o0
    on1, ot1 = o1
    mid = jnp.concatenate([ot0, ot1], axis=0).T
    lane = lax.broadcasted_iota(jnp.int32, (_SQ, 128), 1)
    rm = jnp.where(lane < 64, r0, r1)
    o = jnp.concatenate([on0 * r0, mid * rm, on1 * r1], axis=1)
    return jnp.dot(o.astype(_BF16), wo, preferred_element_type=_F32)


class _Awaited:
    def __init__(self, ref, wait):
        self._ref, self._wait = ref, wait

    def __getitem__(self, idx):
        if self._wait is not None:
            self._wait()
            self._wait = None
        return self._ref[idx]


def _task(x, wq, k, v, wo):
    qa0, qa1 = _qproj(x[0][...], wq[0][...])
    qb0, qb1 = _qproj(x[1][...], wq[1][...])
    sa0 = _scores(qa0, k[0], 0)
    sb0 = _scores(qb0, k[1], 0)
    pa0, ra0 = _softmax(sa0)
    sa1 = _scores(qa1, k[0], 1)
    oa0 = _pv(pa0, v[0], 0)
    pb0, rb0 = _softmax(sb0)
    ob0 = _pv(pb0, v[1], 0)
    pa1, ra1 = _softmax(sa1)
    sb1 = _scores(qb1, k[1], 1)
    oa1 = _pv(pa1, v[0], 1)
    pb1, rb1 = _softmax(sb1)
    ob1 = _pv(pb1, v[1], 1)
    ya = _oproj(oa0, oa1, ra0, ra1, wo[0][...])
    yb = _oproj(ob0, ob1, rb0, rb1, wo[1][...])
    return ya, yb


def _kernel(xa_h, xb_h, ka_h, va_h, kb_h, vb_h, wqa_h, wqb_h, woa_h, wob_h, out_h,
            x_v, wq_v, wo_v, k_v, v_v, acc, out_v,
            sem_x, sem_wq, sem_wo, sem_k, sem_v, sem_o):
    x_h, k_h, v_h = (xa_h, xb_h), (ka_h, kb_h), (va_h, vb_h)
    wq_h, wo_h = (wqa_h, wqb_h), (woa_h, wob_h)
    iters_per_pair = _B // _T

    def rows(hp):
        return pl.ds(pl.multiple_of(hp * _PW, _PW), _PW)

    def x_copy(b, g):
        return pltpu.make_async_copy(x_h[g].at[b], x_v.at[g, b], sem_x.at[g, b])

    def wq_copy(hp, g):
        return pltpu.make_async_copy(
            wq_h[g].at[:, rows(hp)], wq_v.at[hp % 2, g], sem_wq.at[hp % 2, g])

    def wo_copy(hp, g):
        return pltpu.make_async_copy(
            wo_h[g].at[rows(hp), :], wo_v.at[hp % 2, g], sem_wo.at[hp % 2, g])

    def k_copy(t, slot, g):
        return pltpu.make_async_copy(
            k_h[g].at[t % _B, rows(t // _B), :], k_v.at[slot, g], sem_k.at[slot, g])

    def v_copy(t, slot, g):
        return pltpu.make_async_copy(
            v_h[g].at[t % _B, rows(t // _B), :], v_v.at[slot, g], sem_v.at[slot, g])

    def o_copy(b):
        return pltpu.make_async_copy(out_v.at[b], out_h.at[b], sem_o.at[b])

    for g in range(2):
        x_copy(0, g).start()
        wq_copy(0, g).start()
    for g in range(2):
        k_copy(0, 0, g).start()
    for g in range(2):
        v_copy(0, 0, g).start()
    for g in range(2):
        wo_copy(0, g).start()
    for t in range(1, _NS - 1):
        for g in range(2):
            x_copy(t, g).start()
        for g in range(2):
            k_copy(t, t, g).start()
        for g in range(2):
            v_copy(t, t, g).start()

    def body(i, carry):
        hp = i // iters_per_pair
        ih = i % iters_per_pair
        ws = hp % 2
        for j in range(_T):
            t = i * _T + j
            b = ih * _T + j
            slot = j % _NS
            tn = t + _NS - 1
            nslot = (j + _NS - 1) % _NS

            @pl.when(tn < _NTASK)
            def _():
                tc = jnp.minimum(tn, _NTASK - 1)
                for g in range(2):
                    k_copy(tc, nslot, g).start()
                for g in range(2):
                    v_copy(tc, nslot, g).start()

            @pl.when(tn < _B)
            def _():
                tc = jnp.minimum(tn, _B - 1)
                for g in range(2):
                    x_copy(tc, g).start()

            if j == 0:
                @pl.when(jnp.logical_and(ih == 0, hp + 1 < _NP))
                def _():
                    hc = jnp.minimum(hp + 1, _NP - 1)
                    for g in range(2):
                        wq_copy(hc, g).start()
                        wo_copy(hc, g).start()

            def wait_x(g):
                @pl.when(hp == 0)
                def _():
                    x_copy(b, g).wait()

            def wait_wq(g):
                if j == 0:
                    @pl.when(ih == 0)
                    def _():
                        wq_copy(hp, g).wait()

            def wait_wo(g):
                if j == 0:
                    @pl.when(ih == 0)
                    def _():
                        wo_copy(hp, g).wait()

            def wait_k(g):
                k_copy(t, slot, g).wait()

            def wait_v(g):
                v_copy(t, slot, g).wait()

            def awaited(ref, wait):
                return [_Awaited(ref(g), functools.partial(wait, g)) for g in range(2)]

            ya, yb = _task(
                awaited(lambda g: x_v.at[g, b], wait_x),
                awaited(lambda g: wq_v.at[ws, g], wait_wq),
                awaited(lambda g: k_v.at[slot, g], wait_k),
                awaited(lambda g: v_v.at[slot, g], wait_v),
                awaited(lambda g: wo_v.at[ws, g], wait_wo))

            for g, y in enumerate((ya, yb)):
                y = y + jnp.where(hp == 0, 0.0, acc[g, b])
                acc[g, b] = y
                out_v[b, :, g * _D:(g + 1) * _D] = y.astype(out_v.dtype)

            @pl.when(hp == _NP - 1)
            def _():
                o_copy(b).start()
        return carry

    lax.fori_loop(0, _NTASK // _T, body, 0)
    for b in range(_B):
        o_copy(b).wait()


@jax.jit
def pallas_concat_heads__gqa_block_cached__gqa_block_cached__near_ridge_kernel(
    A_x: jax.Array,
    A_k_cache: jax.Array,
    A_v_cache: jax.Array,
    A_wq: jax.Array,
    A_wo: jax.Array,
    B_x: jax.Array,
    B_k_cache: jax.Array,
    B_v_cache: jax.Array,
    B_wq: jax.Array,
    B_wo: jax.Array,
):
    def keys_minor(cache):
        return jnp.swapaxes(cache, 2, 3).reshape(_B, _H * _DH, _SK)

    in_hbm = pl.BlockSpec(memory_space=pl.ANY)
    return pl.pallas_call(
        _kernel,
        in_specs=[in_hbm] * 10,
        out_specs=in_hbm,
        out_shape=jax.ShapeDtypeStruct((_B, _SQ, 2 * _D), A_x.dtype),
        scratch_shapes=[
            pltpu.VMEM((2, _B, _SQ, _D), _BF16),
            pltpu.VMEM((2, 2, _D, _PW), _BF16),
            pltpu.VMEM((2, 2, _PW, _D), _BF16),
            pltpu.VMEM((_NS, 2, _PW, _SK), _BF16),
            pltpu.VMEM((_NS, 2, _PW, _SK), _BF16),
            pltpu.VMEM((2, _B, _SQ, _D), _F32),
            pltpu.VMEM((_B, _SQ, 2 * _D), _BF16),
            pltpu.SemaphoreType.DMA((2, _B)),
            pltpu.SemaphoreType.DMA((2, 2)),
            pltpu.SemaphoreType.DMA((2, 2)),
            pltpu.SemaphoreType.DMA((_NS, 2)),
            pltpu.SemaphoreType.DMA((_NS, 2)),
            pltpu.SemaphoreType.DMA((_B,)),
        ],
        compiler_params=pltpu.CompilerParams(
            vmem_limit_bytes=120 * 1024 * 1024,
            disable_bounds_checks=True,
            flags={"XLA_TPU_RESCHEDULE_DMA_DONES": True},
        ),
    )(A_x, B_x, keys_minor(A_k_cache), keys_minor(A_v_cache),
      keys_minor(B_k_cache), keys_minor(B_v_cache), A_wq, B_wq, A_wo, B_wo)
```

```python
import functools

import jax
import jax.numpy as jnp
from jax import lax
import jax.experimental.pallas as pl
import jax.experimental.pallas.tpu as pltpu

_B, _SQ, _D, _H, _SK, _DH = 8, 240, 640, 32, 1024, 192
_NP = _H // 2
_PW = 2 * _DH
_NTASK = _NP * _B
_T = 4
_NS = 2
_IPP = _B // _T
_LOG_IPP = _IPP.bit_length() - 1
_W_AT = 2

_LOG2E = 1.4426950408889634
_QSCALE = 0.072265625 * _LOG2E
_NT = (((1,), (1,)), ((), ()))
_F32 = jnp.float32
_BF16 = jnp.bfloat16


def _qproj(x, wq):
    q = jnp.dot(x, wq, preferred_element_type=_F32) * _QSCALE
    lane = lax.broadcasted_iota(jnp.int32, (_SQ, 128), 1)
    t0, t1, t2 = q[:, 0:128], q[:, 128:256], q[:, 256:384]
    q0 = jnp.concatenate([t0, jnp.where(lane < 64, t1, 0.0)], axis=1)
    q1 = jnp.concatenate([jnp.where(lane >= 64, t1, 0.0), t2], axis=1)
    return q0.astype(_BF16), q1.astype(_BF16)


def _scores(q, k_ref, h):
    return jnp.dot(q, k_ref[128 * h:128 * h + 256], preferred_element_type=_F32)


def _softmax(s):
    m = jnp.max(s, axis=-1, keepdims=True)
    p = jnp.exp2(s - m).astype(_BF16)
    l = jnp.sum(p.astype(_F32), axis=-1, keepdims=True)
    return p, pl.reciprocal(l, approx=True)


def _pv(p, v_ref, h):
    if h == 0:
        vn, vt = v_ref[0:128], v_ref[128:192]
    else:
        vt, vn = v_ref[192:256], v_ref[256:384]
    on = lax.dot_general(p, vn, _NT, preferred_element_type=_F32)
    ot = lax.dot_general(vt, p, _NT, preferred_element_type=_F32)
    return on, ot


def _oproj(o0, o1, r0, r1, wo):
    on0, ot0 = o0
    on1, ot1 = o1
    mid = jnp.concatenate([ot0, ot1], axis=0).T
    lane = lax.broadcasted_iota(jnp.int32, (_SQ, 128), 1)
    rm = jnp.where(lane < 64, r0, r1)
    o = jnp.concatenate([on0 * r0, mid * rm, on1 * r1], axis=1)
    return jnp.dot(o.astype(_BF16), wo, preferred_element_type=_F32)


class _Awaited:
    def __init__(self, ref, wait):
        self._ref, self._wait = ref, wait

    def __getitem__(self, idx):
        if self._wait is not None:
            self._wait()
            self._wait = None
        return self._ref[idx]


def _task(x, wq, k, v, wo, prefetch_weights):
    qa0, qa1 = _qproj(x[0][...], wq[0][...])
    prefetch_weights()
    qb0, qb1 = _qproj(x[1][...], wq[1][...])
    sa0 = _scores(qa0, k[0], 0)
    sb0 = _scores(qb0, k[1], 0)
    pa0, ra0 = _softmax(sa0)
    sa1 = _scores(qa1, k[0], 1)
    oa0 = _pv(pa0, v[0], 0)
    pb0, rb0 = _softmax(sb0)
    ob0 = _pv(pb0, v[1], 0)
    pa1, ra1 = _softmax(sa1)
    sb1 = _scores(qb1, k[1], 1)
    oa1 = _pv(pa1, v[0], 1)
    pb1, rb1 = _softmax(sb1)
    ob1 = _pv(pb1, v[1], 1)
    ya = _oproj(oa0, oa1, ra0, ra1, wo[0][...])
    yb = _oproj(ob0, ob1, rb0, rb1, wo[1][...])
    return ya, yb


def _kernel(xa_h, xb_h, ka_h, va_h, kb_h, vb_h, wqa_h, wqb_h, woa_h, wob_h, out_h,
            x_v, wq_v, wo_v, k_v, v_v, acc, out_v,
            sem_x, sem_wq, sem_wo, sem_k, sem_v, sem_o):
    x_h, k_h, v_h = (xa_h, xb_h), (ka_h, kb_h), (va_h, vb_h)
    wq_h, wo_h = (wqa_h, wqb_h), (woa_h, wob_h)

    def rows(hp):
        return pl.ds(pl.multiple_of(hp * _PW, _PW), _PW)

    def x_copy(b, g):
        return pltpu.make_async_copy(x_h[g].at[b], x_v.at[g, b], sem_x.at[g, b])

    def wq_copy(hp, g):
        return pltpu.make_async_copy(
            wq_h[g].at[:, rows(hp)], wq_v.at[hp & 1, g], sem_wq.at[hp & 1, g])

    def wo_copy(hp, g):
        return pltpu.make_async_copy(
            wo_h[g].at[rows(hp), :], wo_v.at[hp & 1, g], sem_wo.at[hp & 1, g])

    def k_copy(t, slot, g):
        return pltpu.make_async_copy(
            k_h[g].at[t & (_B - 1), rows(t >> 3), :], k_v.at[slot, g], sem_k.at[slot, g])

    def v_copy(t, slot, g):
        return pltpu.make_async_copy(
            v_h[g].at[t & (_B - 1), rows(t >> 3), :], v_v.at[slot, g], sem_v.at[slot, g])

    def o_copy(b, g):
        return pltpu.make_async_copy(
            out_v.at[g, b], out_h.at[b, :, g * _D:(g + 1) * _D], sem_o.at[g, b])

    first = [
        [x_copy(0, 0), wq_copy(0, 0)],
        [x_copy(0, 1), wq_copy(0, 1)],
        [k_copy(0, 0, 0)],
        [k_copy(0, 0, 1)],
        [v_copy(0, 0, 0)],
        [v_copy(0, 0, 1)],
        [wo_copy(0, 0)],
        [wo_copy(0, 1)],
    ]

    def issue(step, carry):
        for n, copies in enumerate(first):
            @pl.when(step == n)
            def _():
                for copy in copies:
                    copy.start()
        return carry

    lax.fori_loop(0, len(first), issue, 0)
    acc[...] = jnp.zeros(acc.shape, acc.dtype)

    def body(i, carry):
        hp = lax.shift_right_logical(i, _LOG_IPP)
        ih = lax.bitwise_and(i, _IPP - 1)
        ws = lax.bitwise_and(hp, 1)
        more_pairs = hp + 1 < _NP
        hn = jnp.minimum(hp + 1, _NP - 1)
        for j in range(_T):
            t = i * _T + j
            b = ih * _T + j
            slot = j % _NS
            tn = t + 1
            nslot = (j + 1) % _NS

            @pl.when(tn < _B)
            def _():
                for g in range(2):
                    x_copy(jnp.minimum(tn, _B - 1), g).start()

            @pl.when(tn < _NTASK)
            def _():
                tc = jnp.minimum(tn, _NTASK - 1)
                for g in range(2):
                    k_copy(tc, nslot, g).start()
                for g in range(2):
                    v_copy(tc, nslot, g).start()

            def prefetch_weights():
                if j == _W_AT % _T:
                    @pl.when(jnp.logical_and(ih == _W_AT // _T, more_pairs))
                    def _():
                        for g in range(2):
                            wq_copy(hn, g).start()
                            wo_copy(hn, g).start()

            def wait_x(g):
                @pl.when(hp == 0)
                def _():
                    x_copy(b, g).wait()

            def wait_wq(g):
                if j == 0:
                    @pl.when(ih == 0)
                    def _():
                        wq_copy(hp, g).wait()

            def wait_wo(g):
                if j == 0:
                    @pl.when(ih == 0)
                    def _():
                        wo_copy(hp, g).wait()

            def wait_k(g):
                k_copy(t, slot, g).wait()

            def wait_v(g):
                v_copy(t, slot, g).wait()

            def awaited(ref, wait):
                return [_Awaited(ref(g), functools.partial(wait, g)) for g in range(2)]

            ya, yb = _task(
                awaited(lambda g: x_v.at[g, b], wait_x),
                awaited(lambda g: wq_v.at[ws, g], wait_wq),
                awaited(lambda g: k_v.at[slot, g], wait_k),
                awaited(lambda g: v_v.at[slot, g], wait_v),
                awaited(lambda g: wo_v.at[ws, g], wait_wo),
                prefetch_weights)

            for g, y in enumerate((ya, yb)):
                y = y + acc[g, b]
                acc[g, b] = y
                out_v[g, b] = y.astype(out_v.dtype)

                @pl.when(hp == _NP - 1)
                def _():
                    o_copy(b, g).start()
        return carry

    lax.fori_loop(0, _NTASK // _T, body, 0)
    for b in range(_B):
        for g in range(2):
            o_copy(b, g).wait()


@jax.jit
def pallas_concat_heads__gqa_block_cached__gqa_block_cached__near_ridge_kernel(
    A_x: jax.Array,
    A_k_cache: jax.Array,
    A_v_cache: jax.Array,
    A_wq: jax.Array,
    A_wo: jax.Array,
    B_x: jax.Array,
    B_k_cache: jax.Array,
    B_v_cache: jax.Array,
    B_wq: jax.Array,
    B_wo: jax.Array,
):
    def keys_minor(cache):
        return jnp.swapaxes(cache, 2, 3).reshape(_B, _H * _DH, _SK)

    in_hbm = pl.BlockSpec(memory_space=pl.ANY)
    return pl.pallas_call(
        _kernel,
        in_specs=[in_hbm] * 10,
        out_specs=in_hbm,
        out_shape=jax.ShapeDtypeStruct((_B, _SQ, 2 * _D), A_x.dtype),
        scratch_shapes=[
            pltpu.VMEM((2, _B, _SQ, _D), _BF16),
            pltpu.VMEM((2, 2, _D, _PW), _BF16),
            pltpu.VMEM((2, 2, _PW, _D), _BF16),
            pltpu.VMEM((_NS, 2, _PW, _SK), _BF16),
            pltpu.VMEM((_NS, 2, _PW, _SK), _BF16),
            pltpu.VMEM((2, _B, _SQ, _D), _F32),
            pltpu.VMEM((2, _B, _SQ, _D), _BF16),
            pltpu.SemaphoreType.DMA((2, _B)),
            pltpu.SemaphoreType.DMA((2, 2)),
            pltpu.SemaphoreType.DMA((2, 2)),
            pltpu.SemaphoreType.DMA((_NS, 2)),
            pltpu.SemaphoreType.DMA((_NS, 2)),
            pltpu.SemaphoreType.DMA((2, _B)),
        ],
        compiler_params=pltpu.CompilerParams(
            vmem_limit_bytes=100 * 1024 * 1024,
            flags={"XLA_TPU_RESCHEDULE_DMA_DONES": True},
        ),
    )(A_x, B_x, keys_minor(A_k_cache), keys_minor(A_v_cache),
      keys_minor(B_k_cache), keys_minor(B_v_cache), A_wq, B_wq, A_wo, B_wo)
```
